```python
import os as _os
_os.environ.setdefault('JAX_PLATFORMS', 'cpu')
import jax
import jax.numpy as jnp

def _softmax(x, axis=-1):
    return jax.nn.softmax(x, axis=axis)

def _gelu(x):
    return jax.nn.gelu(x, approximate=True)

def _silu(x):
    return jax.nn.silu(x)

def _sigmoid(x):
    return jax.nn.sigmoid(x)

def _layernorm(x, axis=-1, eps=1e-05):
    m = jnp.mean(x, axis=axis, keepdims=True)
    v = jnp.var(x, axis=axis, keepdims=True)
    return (x - m) / jnp.sqrt(v + eps)

def _scatter_add(tgt, idx, src, axis=0):
    return tgt.at[idx].add(src)

def _segment_sum(src, seg, n):
    return jax.ops.segment_sum(src, seg, n)

class _Rng:

    def __init__(self, key):
        self._k = key

    def _next(self):
        self._k, sub = jax.random.split(self._k)
        return sub

    def normal(self, shape):
        return jax.random.normal(self._next(), shape, dtype=jnp.bfloat16)

    def randint(self, lo, hi, shape):
        return jax.random.randint(self._next(), shape, lo, hi, dtype=jnp.int32)

    def uniform(self, shape, lo=0.0, hi=1.0):
        return jax.random.uniform(self._next(), shape, jnp.bfloat16, lo, hi)

    def permutation(self, n):
        return jax.random.permutation(self._next(), n)
kernel_name = 'adaLN_cond__mha_block_cached__geglu_ffn__prompt'

def setup_inputs():
    _rng = _Rng(jax.random.key(int.from_bytes(__import__("os").urandom(4), "little")))
    _w = lambda a: (lambda t: t.astype(jnp.bfloat16) if jnp.issubdtype(t.dtype, jnp.floating) else t)(jnp.asarray(a))

    def _A_setup():
        B, Sq, D = (1, 2048, 512)
        H, Sk, Dh = (32, 2048, 128)
        return {'x': _w((lambda *s: _rng.normal(s) * 0.05)(B, Sq, D)), 'k_cache': _w((lambda *s: _rng.normal(s) * 3.2)(B, H, Sk, Dh)), 'v_cache': _w((lambda *s: _rng.normal(s) * 0.4)(B, H, Sk, Dh)), 'wq': _w((lambda *s: _rng.normal(s) * 1.6)(D, H * Dh) * D ** (-0.5)), 'wo': _w((lambda *s: _rng.normal(s) * 0.4)(H * Dh, D) * (H * Dh) ** (-0.5))}
    _A_in = _A_setup()

    def _B_setup():
        B, S, D, F = (1, 2048, 512, 1792)
        return {'x': _w((lambda *s: _rng.normal(s) * 0.05)(B, S, D)), 'w_gate': _w((lambda *s: _rng.normal(s) * 0.05)(D, F)), 'w_up': _w((lambda *s: _rng.normal(s) * 0.05)(D, F)), 'w_down': _w((lambda *s: _rng.normal(s) * 0.05)(F, D))}
    _B_in = _B_setup()
    return {'A_x': _A_in['x'], 'A_k_cache': _A_in['k_cache'], 'A_v_cache': _A_in['v_cache'], 'A_wq': _A_in['wq'], 'A_wo': _A_in['wo'], 'B_x': _B_in['x'], 'B_w_gate': _B_in['w_gate'], 'B_w_up': _B_in['w_up'], 'B_w_down': _B_in['w_down'], 'c': _w((lambda *s: _rng.normal(s) * 0.05)(1, 512) * 8.0), 'w_mod': _w((lambda *s: _rng.normal(s) * 0.05)(512, 6 * 512) * 512 ** (-0.5) * 8.0)}

def reference(A_x, A_k_cache, A_v_cache, A_wq, A_wo, B_x, B_w_gate, B_w_up, B_w_down, c, w_mod):

    def _A_ref(x, k_cache, v_cache, wq, wo):
        B, Sq, D = x.shape
        H, Dh = (32, 128)
        q = (lambda x, *d: x.transpose(*d))((x @ wq).reshape(B, Sq, H, Dh), 0, 2, 1, 3)
        scores = jnp.einsum('bhqd,bhkd->bhqk', q, k_cache) * Dh ** (-0.5)
        p = _softmax(scores, axis=-1)
        o = jnp.einsum('bhqk,bhkd->bhqd', p, v_cache)
        return (lambda x, *d: x.transpose(*d))(o, 0, 2, 1, 3).reshape(B, Sq, H * Dh) @ wo

    def _B_ref(x, w_gate, w_up, w_down):
        return _gelu(x @ w_gate) * (x @ w_up) @ w_down
    x = A_x
    mod = (_silu(c) @ w_mod).reshape(c.shape[0], 6, 1, -1)
    sa, ca, ga, sb, cb, gb = (mod[:, 0].copy(), mod[:, 1].copy(), mod[:, 2].copy(), mod[:, 3].copy(), mod[:, 4].copy(), mod[:, 5].copy())
    h = _layernorm(x, axis=-1) * (1 + ca) + sa
    x = x + ga * _A_ref(h, A_k_cache, A_v_cache, A_wq, A_wo)
    h = _layernorm(x, axis=-1) * (1 + cb) + sb
    x = x + gb * _B_ref(h, B_w_gate, B_w_up, B_w_down)
    return x
```

```python
import functools

import jax
import jax.numpy as jnp
import jax.experimental.pallas as pl
import jax.experimental.pallas.tpu as pltpu

F32 = jnp.float32
BF16 = jnp.bfloat16

TQ = 512


def _layernorm_f32(x, eps=1e-5):
    m = jnp.mean(x, axis=-1, keepdims=True)
    xc = x - m
    v = jnp.mean(xc * xc, axis=-1, keepdims=True)
    return xc * jax.lax.rsqrt(v + eps)


def _gelu_tanh(x):
    c0 = 0.7978845608028654
    return 0.5 * x * (1.0 + jnp.tanh(c0 * (x + 0.044715 * (x * x * x))))


def _kernel(c_ref, wmod_ref, x_ref, k_ref, v_ref, wq_ref, wo_ref,
            wg_ref, wu_ref, wd_ref, o_ref, mod_scr, h_scr, acc_scr, *, n_heads, d_model, q_scale):
    qi = pl.program_id(0)
    hd = pl.program_id(1)

    @pl.when(jnp.logical_and(qi == 0, hd == 0))
    def _():
        cc = c_ref[...].astype(F32)
        s = cc * jax.nn.sigmoid(cc)
        mod_scr[...] = jnp.dot(s.astype(BF16), wmod_ref[...], preferred_element_type=F32)

    @pl.when(hd == 0)
    def _():
        x = x_ref[...].astype(F32)
        sa = mod_scr[:, 0 * d_model:1 * d_model]
        ca = mod_scr[:, 1 * d_model:2 * d_model]
        h_scr[...] = (_layernorm_f32(x) * (1.0 + ca) + sa).astype(BF16)

    q = jnp.dot(h_scr[...], wq_ref[...], preferred_element_type=F32)
    q = (q * q_scale).astype(BF16)
    s = jax.lax.dot_general(q, k_ref[...], (((1,), (1,)), ((), ())),
                            preferred_element_type=F32)
    m = jnp.max(s, axis=-1, keepdims=True)
    p = jnp.exp2(s - m)
    l = jnp.sum(p, axis=-1, keepdims=True)
    o = jnp.dot(p.astype(BF16), v_ref[...], preferred_element_type=F32)
    o = (o / l).astype(BF16)
    contrib = jnp.dot(o, wo_ref[...], preferred_element_type=F32)

    @pl.when(hd == 0)
    def _():
        acc_scr[...] = contrib

    @pl.when(hd > 0)
    def _():
        acc_scr[...] += contrib

    @pl.when(hd == n_heads - 1)
    def _():
        x = x_ref[...].astype(F32)
        ga = mod_scr[:, 2 * d_model:3 * d_model]
        sb = mod_scr[:, 3 * d_model:4 * d_model]
        cb = mod_scr[:, 4 * d_model:5 * d_model]
        gb = mod_scr[:, 5 * d_model:6 * d_model]
        x1 = x + ga * acc_scr[...]
        h2 = (_layernorm_f32(x1) * (1.0 + cb) + sb).astype(BF16)
        g = jnp.dot(h2, wg_ref[...], preferred_element_type=F32)
        u = jnp.dot(h2, wu_ref[...], preferred_element_type=F32)
        a = (_gelu_tanh(g) * u).astype(BF16)
        y = jnp.dot(a, wd_ref[...], preferred_element_type=F32)
        o_ref[...] = (x1 + gb * y).astype(o_ref.dtype)


@jax.jit
def pallas_adaLN_cond__mha_block_cached__geglu_ffn__prompt_kernel(
    A_x: jax.Array,
    A_k_cache: jax.Array,
    A_v_cache: jax.Array,
    A_wq: jax.Array,
    A_wo: jax.Array,
    B_x: jax.Array,
    B_w_gate: jax.Array,
    B_w_up: jax.Array,
    B_w_down: jax.Array,
    c: jax.Array,
    w_mod: jax.Array,
):
    B, Sq, D = A_x.shape
    _, H, Sk, Dh = A_k_cache.shape
    F = B_w_gate.shape[1]
    assert B == 1 and Sq % TQ == 0
    q_scale = float(Dh) ** -0.5 * 1.4426950408889634

    x2 = A_x.reshape(Sq, D)
    k3 = A_k_cache.reshape(H, Sk, Dh)
    v3 = A_v_cache.reshape(H, Sk, Dh)

    kern = functools.partial(_kernel, n_heads=H, d_model=D, q_scale=q_scale)
    const = lambda qi, hd: (0, 0)
    out = pl.pallas_call(
        kern,
        grid=(Sq // TQ, H),
        in_specs=[
            pl.BlockSpec((1, D), const),
            pl.BlockSpec((D, 6 * D), const),
            pl.BlockSpec((TQ, D), lambda qi, hd: (qi, 0)),
            pl.BlockSpec((None, Sk, Dh), lambda qi, hd: (hd, 0, 0)),
            pl.BlockSpec((None, Sk, Dh), lambda qi, hd: (hd, 0, 0)),
            pl.BlockSpec((D, Dh), lambda qi, hd: (0, hd)),
            pl.BlockSpec((Dh, D), lambda qi, hd: (hd, 0)),
            pl.BlockSpec((D, F), const),
            pl.BlockSpec((D, F), const),
            pl.BlockSpec((F, D), const),
        ],
        out_specs=pl.BlockSpec((TQ, D), lambda qi, hd: (qi, 0)),
        out_shape=jax.ShapeDtypeStruct((Sq, D), A_x.dtype),
        scratch_shapes=[
            pltpu.VMEM((1, 6 * D), F32),
            pltpu.VMEM((TQ, D), BF16),
            pltpu.VMEM((TQ, D), F32),
        ],
        compiler_params=pltpu.CompilerParams(
            dimension_semantics=("arbitrary", "arbitrary"),
            vmem_limit_bytes=100 * 1024 * 1024,
        ),
    )(c, w_mod, x2, k3, v3, A_wq, A_wo, B_w_gate, B_w_up, B_w_down)
    return out.reshape(B, Sq, D)
```

```python
import functools

import jax
import jax.numpy as jnp
import jax.experimental.pallas as pl
import jax.experimental.pallas.tpu as pltpu

F32 = jnp.float32
BF16 = jnp.bfloat16

TQ = 512
HPS = 4


def _layernorm_f32(x, eps=1e-5):
    m = jnp.mean(x, axis=-1, keepdims=True)
    xc = x - m
    v = jnp.mean(xc * xc, axis=-1, keepdims=True)
    return xc * jax.lax.rsqrt(v + eps)


def _gelu_tanh(x):
    c0 = 0.7978845608028654
    return 0.5 * x * (1.0 + jnp.tanh(c0 * (x + 0.044715 * (x * x * x))))


def _kernel(c_ref, wmod_ref, x_ref, k_ref, v_ref, wq_ref, wo_ref,
            wg_hbm, wu_hbm, wd_hbm, o_ref,
            mod_scr, h_scr, acc_scr, wg_ref, wu_ref, wd_ref, sems,
            *, n_steps, d, dh, q_scale):
    qi = pl.program_id(0)
    hs = pl.program_id(1)

    def w_copies():
        pairs = ((wg_hbm, wg_ref), (wu_hbm, wu_ref), (wd_hbm, wd_ref))
        return [pltpu.make_async_copy(src, dst, sems.at[i]) for i, (src, dst) in enumerate(pairs)]

    @pl.when(jnp.logical_and(qi == 0, hs == 0))
    def _():
        for cp in w_copies():
            cp.start()
        cc = c_ref[...].astype(F32)
        s = cc * jax.nn.sigmoid(cc)
        mod_scr[...] = jnp.dot(s.astype(BF16), wmod_ref[...], preferred_element_type=F32)

    @pl.when(hs == 0)
    def _():
        x = x_ref[...].astype(F32)
        sa = mod_scr[:, 0 * d:1 * d]
        ca = mod_scr[:, 1 * d:2 * d]
        h_scr[...] = (_layernorm_f32(x) * (1.0 + ca) + sa).astype(BF16)
        acc_scr[...] = jnp.zeros_like(acc_scr)

    q_all = jnp.dot(h_scr[...], wq_ref[...], preferred_element_type=F32)
    q_all = (q_all * q_scale).astype(BF16)
    outs = []
    for j in range(HPS):
        q = q_all[:, j * dh:(j + 1) * dh]
        s = jax.lax.dot_general(q, k_ref[j], (((1,), (1,)), ((), ())),
                                preferred_element_type=F32)
        m = jnp.max(s, axis=-1, keepdims=True)
        p = jnp.exp2(s - m)
        l = jnp.sum(p, axis=-1, keepdims=True)
        o = jnp.dot(p.astype(BF16), v_ref[j], preferred_element_type=F32)
        outs.append((o / l).astype(BF16))
    o_all = jnp.concatenate(outs, axis=-1)
    contrib = jnp.dot(o_all, wo_ref[...], preferred_element_type=F32)

    acc_scr[...] += contrib

    @pl.when(hs == n_steps - 1)
    def _():
        @pl.when(qi == 0)
        def _():
            for cp in w_copies():
                cp.wait()

        x = x_ref[...].astype(F32)
        ga = mod_scr[:, 2 * d:3 * d]
        sb = mod_scr[:, 3 * d:4 * d]
        cb = mod_scr[:, 4 * d:5 * d]
        gb = mod_scr[:, 5 * d:6 * d]
        x1 = x + ga * acc_scr[...]
        h2 = (_layernorm_f32(x1) * (1.0 + cb) + sb).astype(BF16)
        g = jnp.dot(h2, wg_ref[...], preferred_element_type=F32)
        u = jnp.dot(h2, wu_ref[...], preferred_element_type=F32)
        a = (_gelu_tanh(g) * u).astype(BF16)
        y = jnp.dot(a, wd_ref[...], preferred_element_type=F32)
        o_ref[...] = (x1 + gb * y).astype(o_ref.dtype)


@jax.jit
def pallas_adaLN_cond__mha_block_cached__geglu_ffn__prompt_kernel(
    A_x: jax.Array,
    A_k_cache: jax.Array,
    A_v_cache: jax.Array,
    A_wq: jax.Array,
    A_wo: jax.Array,
    B_x: jax.Array,
    B_w_gate: jax.Array,
    B_w_up: jax.Array,
    B_w_down: jax.Array,
    c: jax.Array,
    w_mod: jax.Array,
):
    B, Sq, D = A_x.shape
    _, H, Sk, Dh = A_k_cache.shape
    F = B_w_gate.shape[1]
    assert B == 1 and Sq % TQ == 0 and H % HPS == 0
    q_scale = float(Dh) ** -0.5 * 1.4426950408889634

    x2 = A_x.reshape(Sq, D)
    k3 = A_k_cache.reshape(H, Sk, Dh)
    v3 = A_v_cache.reshape(H, Sk, Dh)

    kern = functools.partial(_kernel, n_steps=H // HPS, d=D, dh=Dh, q_scale=q_scale)
    const = lambda qi, hs: (0, 0)
    out = pl.pallas_call(
        kern,
        grid=(Sq // TQ, H // HPS),
        in_specs=[
            pl.BlockSpec((1, D), const),
            pl.BlockSpec((D, 6 * D), const),
            pl.BlockSpec((TQ, D), lambda qi, hs: (qi, 0)),
            pl.BlockSpec((HPS, Sk, Dh), lambda qi, hs: (hs, 0, 0)),
            pl.BlockSpec((HPS, Sk, Dh), lambda qi, hs: (hs, 0, 0)),
            pl.BlockSpec((D, HPS * Dh), lambda qi, hs: (0, hs)),
            pl.BlockSpec((HPS * Dh, D), lambda qi, hs: (hs, 0)),
            pl.BlockSpec(memory_space=pl.ANY),
            pl.BlockSpec(memory_space=pl.ANY),
            pl.BlockSpec(memory_space=pl.ANY),
        ],
        out_specs=pl.BlockSpec((TQ, D), lambda qi, hs: (qi, 0)),
        out_shape=jax.ShapeDtypeStruct((Sq, D), A_x.dtype),
        scratch_shapes=[
            pltpu.VMEM((1, 6 * D), F32),
            pltpu.VMEM((TQ, D), BF16),
            pltpu.VMEM((TQ, D), F32),
            pltpu.VMEM((D, F), BF16),
            pltpu.VMEM((D, F), BF16),
            pltpu.VMEM((F, D), BF16),
            pltpu.SemaphoreType.DMA((3,)),
        ],
        compiler_params=pltpu.CompilerParams(
            dimension_semantics=("arbitrary", "arbitrary"),
            vmem_limit_bytes=110 * 1024 * 1024,
        ),
    )(c, w_mod, x2, k3, v3, A_wq, A_wo, B_w_gate, B_w_up, B_w_down)
    return out.reshape(B, Sq, D)
```
